```python
import os as _os
_os.environ.setdefault("JAX_PLATFORMS", "cpu")
import jax
import jax.numpy as jnp

def _softmax(x, axis=-1):
    return jax.nn.softmax(x, axis=axis)
def _gelu(x):
    return jax.nn.gelu(x, approximate=True)
def _silu(x):
    return jax.nn.silu(x)
def _sigmoid(x):
    return jax.nn.sigmoid(x)
def _layernorm(x, axis=-1, eps=1e-5):
    m = jnp.mean(x, axis=axis, keepdims=True)
    v = jnp.var(x, axis=axis, keepdims=True)
    return (x - m) / jnp.sqrt(v + eps)
def _scatter_add(tgt, idx, src, axis=0):
    return tgt.at[idx].add(src)
def _segment_sum(src, seg, n):
    return jax.ops.segment_sum(src, seg, n)
class _Rng:
    def __init__(self, key):
        self._k = key
    def _next(self):
        self._k, sub = jax.random.split(self._k)
        return sub
    def normal(self, shape):
        return jax.random.normal(self._next(), shape, dtype=jnp.bfloat16)
    def randint(self, lo, hi, shape):
        return jax.random.randint(self._next(), shape, lo, hi, dtype=jnp.int32)
    def uniform(self, shape, lo=0.0, hi=1.0):
        return jax.random.uniform(self._next(), shape, jnp.bfloat16, lo, hi)
    def permutation(self, n):
        return jax.random.permutation(self._next(), n)


kernel_name = 'standalone__gqa_softmax__decode'

def setup_inputs():
    _rng = _Rng(jax.random.key(int.from_bytes(__import__("os").urandom(4), "little")))
    _w = (lambda a: (lambda t: t.astype(jnp.bfloat16) if jnp.issubdtype(t.dtype, jnp.floating) else t)(jnp.asarray(a)))
    B, Hq, Hkv, Sq, Sk, D = 8, 32, 32, 1, 4096, 128
    return {
        "q": _w((lambda *s: _rng.normal(s) * 0.4)(B, Hq, Sq, D)),
        "k": _w((lambda *s: _rng.normal(s) * 0.4)(B, Hkv, Sk, D)),
        "v": _w((lambda *s: _rng.normal(s) * 0.05)(B, Hkv, Sk, D)),
    }

def reference(q, k, v):
    B, Hq, Sq, D = q.shape
    Hkv = k.shape[1]
    rep = Hq // Hkv
    k = jnp.repeat(k, rep, axis=1)
    v = jnp.repeat(v, rep, axis=1)
    scale = D ** -0.5
    scores = jnp.einsum("bhqd,bhkd->bhqk", q, k) * scale
    p = _softmax(scores, axis=-1)
    return jnp.einsum("bhqk,bhkd->bhqd", p, v)
```

```python
import functools

import jax
import jax.numpy as jnp
from jax import lax
import jax.experimental.pallas as pl
import jax.experimental.pallas.tpu as pltpu


def _kernel(q_ref, k_ref, v_ref, o_ref, *, hb, scale):
    for h in range(hb):
        q = q_ref[h]
        k = k_ref[h]
        v = v_ref[h]
        s = lax.dot_general(q, k, (((1,), (1,)), ((), ())),
                            preferred_element_type=jnp.float32)
        s = s * scale
        m = jnp.max(s, axis=-1, keepdims=True)
        p = jnp.exp(s - m)
        l = jnp.sum(p, axis=-1, keepdims=True)
        o = jnp.dot(p.astype(v.dtype), v, preferred_element_type=jnp.float32)
        o_ref[h] = (o / l).astype(o_ref.dtype)


@jax.jit
def pallas_standalone__gqa_softmax__decode_kernel(
    q: jax.Array,
    k: jax.Array,
    v: jax.Array,
):
    B, Hq, Sq, D = q.shape
    _, Hkv, Sk, _ = k.shape
    rep = Hq // Hkv
    M = rep * Sq
    scale = D ** -0.5
    N = B * Hkv
    q3 = q.reshape(N, M, D)
    k3 = k.reshape(N, Sk, D)
    v3 = v.reshape(N, Sk, D)
    hb = 2
    out = pl.pallas_call(
        functools.partial(_kernel, hb=hb, scale=scale),
        grid=(N // hb,),
        in_specs=[
            pl.BlockSpec((hb, M, D), lambda i: (i, 0, 0)),
            pl.BlockSpec((hb, Sk, D), lambda i: (i, 0, 0)),
            pl.BlockSpec((hb, Sk, D), lambda i: (i, 0, 0)),
        ],
        out_specs=pl.BlockSpec((hb, M, D), lambda i: (i, 0, 0)),
        out_shape=jax.ShapeDtypeStruct((N, M, D), q.dtype),
        compiler_params=pltpu.CompilerParams(
            dimension_semantics=("arbitrary",),
            vmem_limit_bytes=64 * 1024 * 1024,
        ),
    )(q3, k3, v3)
    return out.reshape(B, Hq, Sq, D)
```

```python
import functools

import jax
import jax.numpy as jnp
from jax import lax
import jax.experimental.pallas as pl
import jax.experimental.pallas.tpu as pltpu


def _split(total, size):
    out = []
    o = 0
    while o < total:
        r = min(size, total - o)
        out.append((o, r))
        o += r
    return out


def _kernel(q_hbm, k_hbm, v_hbm, o_hbm, qbuf, q32, kbuf, vbuf, o32, obuf,
            qsem, ksem, vsem, osem, *, n, m, sk, nbuf, rows, scale):
    pieces = _split(sk, rows)

    def issue(h, slot):
        for o, r in pieces:
            pltpu.make_async_copy(k_hbm.at[h, pl.ds(o, r)],
                                  kbuf.at[slot, pl.ds(o, r)],
                                  ksem.at[slot]).start(priority=0)
            pltpu.make_async_copy(v_hbm.at[h, pl.ds(o, r)],
                                  vbuf.at[slot, pl.ds(o, r)],
                                  vsem.at[slot]).start(priority=1)

    qc = pltpu.make_async_copy(q_hbm, qbuf, qsem.at[0])
    qc.start()
    for j in range(min(nbuf - 1, n)):
        issue(j, j)
    qc.wait()
    q32[...] = qbuf[...].astype(jnp.float32)

    def body(h, carry):
        slot = lax.rem(h, nbuf)
        nxt = h + nbuf - 1
        nslot = lax.rem(nxt, nbuf)

        @pl.when(nxt < n)
        def _():
            issue(nxt, nslot)

        q = q32[pl.ds(h * m, m), :].astype(kbuf.dtype)
        pltpu.make_async_copy(kbuf.at[slot], kbuf.at[slot], ksem.at[slot]).wait()
        s = lax.dot_general(q, kbuf[slot], (((1,), (1,)), ((), ())),
                            preferred_element_type=jnp.float32)
        s = s * scale
        mx = jnp.max(s, axis=-1, keepdims=True)
        p = jnp.exp(s - mx)
        l = jnp.sum(p, axis=-1, keepdims=True)
        pb = p.astype(vbuf.dtype)
        pltpu.make_async_copy(vbuf.at[slot], vbuf.at[slot], vsem.at[slot]).wait()
        acc = jnp.dot(pb, vbuf[slot], preferred_element_type=jnp.float32)
        o32[pl.ds(h * m, m), :] = acc / l
        return carry

    lax.fori_loop(0, n, body, 0)
    obuf[...] = o32[...].astype(obuf.dtype)
    oc = pltpu.make_async_copy(obuf, o_hbm, osem.at[0])
    oc.start()
    oc.wait()


@jax.jit
def pallas_standalone__gqa_softmax__decode_kernel(
    q: jax.Array,
    k: jax.Array,
    v: jax.Array,
):
    B, Hq, Sq, D = q.shape
    _, Hkv, Sk, _ = k.shape
    rep = Hq // Hkv
    M = rep * Sq
    N = B * Hkv
    scale = D ** -0.5
    nbuf = 3
    rows = 192
    q2 = q.reshape(N * M, D)
    k3 = k.reshape(N, Sk, D)
    v3 = v.reshape(N, Sk, D)
    out = pl.pallas_call(
        functools.partial(_kernel, n=N, m=M, sk=Sk, nbuf=nbuf, rows=rows,
                          scale=scale),
        in_specs=[pl.BlockSpec(memory_space=pl.ANY)] * 3,
        out_specs=pl.BlockSpec(memory_space=pl.ANY),
        out_shape=jax.ShapeDtypeStruct((N * M, D), q.dtype),
        scratch_shapes=[
            pltpu.VMEM((N * M, D), q.dtype),
            pltpu.VMEM((N * M, D), jnp.float32),
            pltpu.VMEM((nbuf, Sk, D), k.dtype),
            pltpu.VMEM((nbuf, Sk, D), v.dtype),
            pltpu.VMEM((N * M, D), jnp.float32),
            pltpu.VMEM((N * M, D), q.dtype),
            pltpu.SemaphoreType.DMA((1,)),
            pltpu.SemaphoreType.DMA((nbuf,)),
            pltpu.SemaphoreType.DMA((nbuf,)),
            pltpu.SemaphoreType.DMA((1,)),
        ],
        compiler_params=pltpu.CompilerParams(
            vmem_limit_bytes=64 * 1024 * 1024),
    )(q2, k3, v3)
    return out.reshape(B, Hq, Sq, D)
```

```python
import functools

import jax
import jax.numpy as jnp
from jax import lax
import jax.experimental.pallas as pl
import jax.experimental.pallas.tpu as pltpu


def _split(total, first, size):
    out = []
    o = 0
    while o < total:
        r = min(size if out else first, total - o)
        out.append((o, r))
        o += r
    return out


def _kernel(q_hbm, k_hbm, v_hbm, o_hbm, qbuf, q32, kbuf, vbuf, o32, obuf,
            qsem, ksem, vsem, osem, *, n, m, sk, nbuf, rows0, rows, scale):
    pieces = _split(sk, rows0, rows)

    def issue(h, slot):
        for o, r in pieces:
            pltpu.make_async_copy(k_hbm.at[h, pl.ds(o, r)],
                                  kbuf.at[slot, pl.ds(o, r)],
                                  ksem.at[slot]).start(priority=0)
            pltpu.make_async_copy(v_hbm.at[h, pl.ds(o, r)],
                                  vbuf.at[slot, pl.ds(o, r)],
                                  vsem.at[slot]).start(priority=1)

    qc = pltpu.make_async_copy(q_hbm, qbuf, qsem.at[0])
    qc.start()
    for j in range(min(nbuf - 1, n)):
        issue(j, j)
    qc.wait()
    q32[...] = qbuf[...].astype(jnp.float32)

    def body(h, carry):
        slot = lax.rem(h, nbuf)
        nxt = h + nbuf - 1
        nslot = lax.rem(nxt, nbuf)

        @pl.when(nxt < n)
        def _():
            issue(nxt, nslot)

        q = q32[pl.ds(h * m, m), :].astype(kbuf.dtype)
        pltpu.make_async_copy(kbuf.at[slot], kbuf.at[slot], ksem.at[slot]).wait()
        s = lax.dot_general(q, kbuf[slot], (((1,), (1,)), ((), ())),
                            preferred_element_type=jnp.float32)
        s = s * scale
        mx = jnp.max(s, axis=-1, keepdims=True)
        p = jnp.exp(s - mx)
        l = jnp.sum(p, axis=-1, keepdims=True)
        pb = p.astype(vbuf.dtype)
        pltpu.make_async_copy(vbuf.at[slot], vbuf.at[slot], vsem.at[slot]).wait()
        acc = jnp.dot(pb, vbuf[slot], preferred_element_type=jnp.float32)
        o32[pl.ds(h * m, m), :] = acc / l
        return carry

    lax.fori_loop(0, n, body, 0)
    obuf[...] = o32[...].astype(obuf.dtype)
    oc = pltpu.make_async_copy(obuf, o_hbm, osem.at[0])
    oc.start()
    oc.wait()


@jax.jit
def pallas_standalone__gqa_softmax__decode_kernel(
    q: jax.Array,
    k: jax.Array,
    v: jax.Array,
):
    B, Hq, Sq, D = q.shape
    _, Hkv, Sk, _ = k.shape
    rep = Hq // Hkv
    M = rep * Sq
    N = B * Hkv
    scale = D ** -0.5
    nbuf = 3
    rows0, rows = 160, 192
    q2 = q.reshape(N * M, D)
    k3 = k.reshape(N, Sk, D)
    v3 = v.reshape(N, Sk, D)
    out = pl.pallas_call(
        functools.partial(_kernel, n=N, m=M, sk=Sk, nbuf=nbuf, rows0=rows0,
                          rows=rows, scale=scale),
        in_specs=[pl.BlockSpec(memory_space=pl.ANY)] * 3,
        out_specs=pl.BlockSpec(memory_space=pl.ANY),
        out_shape=jax.ShapeDtypeStruct((N * M, D), q.dtype),
        scratch_shapes=[
            pltpu.VMEM((N * M, D), q.dtype),
            pltpu.VMEM((N * M, D), jnp.float32),
            pltpu.VMEM((nbuf, Sk, D), k.dtype),
            pltpu.VMEM((nbuf, Sk, D), v.dtype),
            pltpu.VMEM((N * M, D), jnp.float32),
            pltpu.VMEM((N * M, D), q.dtype),
            pltpu.SemaphoreType.DMA((1,)),
            pltpu.SemaphoreType.DMA((nbuf,)),
            pltpu.SemaphoreType.DMA((nbuf,)),
            pltpu.SemaphoreType.DMA((1,)),
        ],
        compiler_params=pltpu.CompilerParams(
            vmem_limit_bytes=64 * 1024 * 1024),
    )(q2, k3, v3)
    return out.reshape(B, Hq, Sq, D)
```

```python
import functools

import jax
import jax.numpy as jnp
from jax import lax
import jax.experimental.pallas as pl
import jax.experimental.pallas.tpu as pltpu

_K_UNITS_4096 = (6, 16, 17, 10, 5, 16, 16, 9, 8, 15, 16, 11, 5, 16, 16, 3, 14, 15, 9, 7, 16, 10)
_V_UNITS_4096 = (5, 18, 14, 15, 7, 10, 15, 15, 2, 15, 15, 16, 9, 9, 16, 12, 4, 16, 16, 2, 14, 11)
_V_LEAD_4096 = 5


def _pieces(sizes):
    out = []
    o = 0
    for r in sizes:
        out.append((o, r))
        o += r
    return out


def _uniform(total, size):
    out = []
    while sum(out) < total:
        out.append(min(size, total - sum(out)))
    return tuple(out)


def _kernel(q_hbm, k_hbm, v_hbm, o_hbm, qbuf, q32, kbuf, vbuf, o32, obuf,
            qsem, ksem, vsem, osem, *, n, m, nbuf, ahead, ksizes, vsizes, lead,
            scale):
    kp, vp = _pieces(ksizes), _pieces(vsizes)
    npc = len(kp)

    def slot_of(h):
        return h % nbuf if isinstance(h, int) else lax.rem(h, nbuf)

    def kstart(h, i):
        o, r = kp[i]
        slot = slot_of(h)
        pltpu.make_async_copy(k_hbm.at[h, pl.ds(o, r)],
                              kbuf.at[slot, pl.ds(o, r)],
                              ksem.at[slot]).start(priority=0)

    def vstart(h, i):
        o, r = vp[i]
        slot = slot_of(h)
        pltpu.make_async_copy(v_hbm.at[h, pl.ds(o, r)],
                              vbuf.at[slot, pl.ds(o, r)],
                              vsem.at[slot]).start(priority=1)

    def issue(h, last):
        for i in range(npc):
            kstart(h, i)
            if i + lead < npc:
                vstart(h, i + lead)
            elif not last:
                vstart(h + 1, i + lead - npc)

    qc = pltpu.make_async_copy(q_hbm, qbuf, qsem.at[0])
    qc.start()
    for i in range(lead):
        vstart(0, i)
    for j in range(min(ahead, n)):
        issue(j, j == n - 1)
    qc.wait()
    q32[...] = qbuf[...].astype(jnp.float32)

    def body(h, carry):
        slot = lax.rem(h, nbuf)
        nxt = h + ahead

        @pl.when(nxt < n - 1)
        def _():
            issue(nxt, False)

        @pl.when(nxt == n - 1)
        def _():
            issue(nxt, True)

        q = q32[pl.ds(h * m, m), :].astype(kbuf.dtype)
        pltpu.make_async_copy(kbuf.at[slot], kbuf.at[slot], ksem.at[slot]).wait()
        s = lax.dot_general(q, kbuf[slot], (((1,), (1,)), ((), ())),
                            preferred_element_type=jnp.float32)
        s = s * scale
        mx = jnp.max(s, axis=-1, keepdims=True)
        p = jnp.exp(s - mx)
        l = jnp.sum(p, axis=-1, keepdims=True)
        pb = p.astype(vbuf.dtype)
        pltpu.make_async_copy(vbuf.at[slot], vbuf.at[slot], vsem.at[slot]).wait()
        acc = jnp.dot(pb, vbuf[slot], preferred_element_type=jnp.float32)
        o32[pl.ds(h * m, m), :] = acc / l
        return carry

    lax.fori_loop(0, n, body, 0)
    obuf[...] = o32[...].astype(obuf.dtype)
    oc = pltpu.make_async_copy(obuf, o_hbm, osem.at[0])
    oc.start()
    oc.wait()


@jax.jit
def pallas_standalone__gqa_softmax__decode_kernel(
    q: jax.Array,
    k: jax.Array,
    v: jax.Array,
):
    B, Hq, Sq, D = q.shape
    _, Hkv, Sk, _ = k.shape
    rep = Hq // Hkv
    M = rep * Sq
    N = B * Hkv
    scale = D ** -0.5
    ahead = 2
    nbuf = ahead + 2
    if Sk == 4096:
        ksizes = tuple(16 * u for u in _K_UNITS_4096)
        vsizes = tuple(16 * u for u in _V_UNITS_4096)
        lead = _V_LEAD_4096
    else:
        ksizes = vsizes = _uniform(Sk, 192)
        lead = 0
    q2 = q.reshape(N * M, D)
    k3 = k.reshape(N, Sk, D)
    v3 = v.reshape(N, Sk, D)
    out = pl.pallas_call(
        functools.partial(_kernel, n=N, m=M, nbuf=nbuf, ahead=ahead,
                          ksizes=ksizes, vsizes=vsizes, lead=lead, scale=scale),
        in_specs=[pl.BlockSpec(memory_space=pl.ANY)] * 3,
        out_specs=pl.BlockSpec(memory_space=pl.ANY),
        out_shape=jax.ShapeDtypeStruct((N * M, D), q.dtype),
        scratch_shapes=[
            pltpu.VMEM((N * M, D), q.dtype),
            pltpu.VMEM((N * M, D), jnp.float32),
            pltpu.VMEM((nbuf, Sk, D), k.dtype),
            pltpu.VMEM((nbuf, Sk, D), v.dtype),
            pltpu.VMEM((N * M, D), jnp.float32),
            pltpu.VMEM((N * M, D), q.dtype),
            pltpu.SemaphoreType.DMA((1,)),
            pltpu.SemaphoreType.DMA((nbuf,)),
            pltpu.SemaphoreType.DMA((nbuf,)),
            pltpu.SemaphoreType.DMA((1,)),
        ],
        compiler_params=pltpu.CompilerParams(
            vmem_limit_bytes=64 * 1024 * 1024),
    )(q2, k3, v3)
    return out.reshape(B, Hq, Sq, D)
```

```python
import functools

import jax
import jax.numpy as jnp
from jax import lax
import jax.experimental.pallas as pl
import jax.experimental.pallas.tpu as pltpu

_K_UNITS_4096 = (
    30, 1, 1, 30, 1, 1, 24, 7, 1, 24, 7, 1, 25, 6, 1, 30, 1, 1, 30, 1, 1, 27, 4, 1,
    30, 1, 1, 30, 1, 1, 30, 1, 1, 30, 1, 1, 30, 1, 1, 30, 1, 1, 30, 1, 1, 30, 1, 1)
_V_UNITS_4096 = (
    5, 24, 3, 3, 26, 2, 5, 25, 3, 5, 24, 2, 4, 26, 3, 4, 24, 3, 5, 26, 1, 3, 27, 2,
    5, 24, 1, 8, 23, 4, 1, 28, 5, 6, 21, 3, 5, 24, 3, 9, 20, 3, 3, 25, 5, 1, 27, 3)
_V_LEAD_4096 = 10
_OFF = 13
_TA = 128


def _pieces(sizes):
    out = []
    o = 0
    for r in sizes:
        out.append((o, r))
        o += r
    return out


def _uniform(total, size):
    out = []
    while sum(out) < total:
        out.append(min(size, total - sum(out)))
    return tuple(out)


def _kernel(q_hbm, k_hbm, v_hbm, o_hbm, qbuf, q32, kbuf, vbuf, o32, obuf,
            qsem, ksem, vsem, osem, *, n, m, sk, nbuf, ahead, ksizes, vsizes,
            lead, off, scale):
    kp, vp = _pieces(ksizes), _pieces(vsizes)
    npc = len(kp)
    body_rows = sk - off
    ta = _TA
    d = kbuf.shape[-1]

    def slot_of(g):
        return g % nbuf if isinstance(g, int) else lax.rem(g, nbuf)

    def start(hbm, buf, sem, queue, g, piece, trunc):
        o, r = piece
        if trunc:
            r = min(r, body_rows - o)
            if r <= 0:
                return
        slot = slot_of(g)
        src = g * sk + off + o
        if not isinstance(src, int):
            src = pl.multiple_of(src, 8)
        pltpu.make_async_copy(hbm.at[pl.ds(src, r)],
                              buf.at[slot, pl.ds(o, r)],
                              sem.at[slot]).start(priority=queue)

    def issue(g, last):
        for i in range(npc):
            start(k_hbm, kbuf, ksem, 0, g, kp[i], last)
            if i + lead < npc:
                start(v_hbm, vbuf, vsem, 1, g, vp[i + lead], last)
            elif not last:
                start(v_hbm, vbuf, vsem, 1, g + 1, vp[i + lead - npc], False)

    qc = pltpu.make_async_copy(q_hbm, qbuf, qsem.at[0])
    qc.start()
    ls = nbuf - 1
    k0c = pltpu.make_async_copy(k_hbm.at[pl.ds(0, off)],
                                kbuf.at[ls, pl.ds(body_rows, off)], ksem.at[ls])
    v0c = pltpu.make_async_copy(v_hbm.at[pl.ds(0, off)],
                                vbuf.at[ls, pl.ds(body_rows, off)], vsem.at[ls])
    k0c.start(priority=0)
    v0c.start(priority=1)
    for i in range(lead):
        start(v_hbm, vbuf, vsem, 1, 0, vp[i], False)
    for j in range(ahead):
        issue(j, False)
    kbuf[ls, pl.ds(sk - ta, ta - off), :] = jnp.zeros((ta - off, d), kbuf.dtype)
    vbuf[ls, pl.ds(sk - ta, ta - off), :] = jnp.zeros((ta - off, d), vbuf.dtype)
    qc.wait()
    q32[...] = qbuf[...].astype(jnp.float32)
    k0c.wait()
    v0c.wait()

    lane = lax.broadcasted_iota(jnp.int32, (m, ta), 1)
    neg = jnp.float32(-jnp.inf)

    def wait_group(buf, sem, slot, h):
        a = buf.at[slot, pl.ds(0, body_rows)]
        pltpu.make_async_copy(a, a, sem.at[slot]).wait()

        @pl.when(h < n - 1)
        def _():
            b = buf.at[slot, pl.ds(body_rows, off)]
            pltpu.make_async_copy(b, b, sem.at[slot]).wait()

    def body(h, carry):
        slot = lax.rem(h, nbuf)
        pslot = lax.rem(h + nbuf - 1, nbuf)
        nxt = h + ahead

        @pl.when(nxt < n - 1)
        def _():
            issue(nxt, False)

        @pl.when(nxt == n - 1)
        def _():
            issue(nxt, True)

        q = q32[pl.ds(h * m, m), :].astype(kbuf.dtype)
        wait_group(kbuf, ksem, slot, h)
        dn = (((1,), (1,)), ((), ()))
        sa = lax.dot_general(q, kbuf[pslot, pl.ds(sk - ta, ta), :], dn,
                             preferred_element_type=jnp.float32)
        sb = lax.dot_general(q, kbuf[slot, pl.ds(0, sk - ta), :], dn,
                             preferred_element_type=jnp.float32)
        sc = lax.dot_general(q, kbuf[slot, pl.ds(sk - ta, ta), :], dn,
                             preferred_element_type=jnp.float32)
        sa = jnp.where(lane >= ta - off, sa * scale, neg)
        sb = sb * scale
        sc = jnp.where(lane < ta - off, sc * scale, neg)
        mx = jnp.maximum(jnp.max(sb, axis=-1, keepdims=True),
                         jnp.max(jnp.maximum(sa, sc), axis=-1, keepdims=True))
        pa = jnp.exp(sa - mx)
        pb = jnp.exp(sb - mx)
        pc = jnp.exp(sc - mx)
        l = (jnp.sum(pb, axis=-1, keepdims=True)
             + jnp.sum(pa + pc, axis=-1, keepdims=True))
        wait_group(vbuf, vsem, slot, h)
        dt = vbuf.dtype
        acc = jnp.dot(pb.astype(dt), vbuf[slot, pl.ds(0, sk - ta), :],
                      preferred_element_type=jnp.float32)
        acc = acc + jnp.dot(pa.astype(dt), vbuf[pslot, pl.ds(sk - ta, ta), :],
                            preferred_element_type=jnp.float32)
        acc = acc + jnp.dot(pc.astype(dt), vbuf[slot, pl.ds(sk - ta, ta), :],
                            preferred_element_type=jnp.float32)
        o32[pl.ds(h * m, m), :] = acc / l
        return carry

    lax.fori_loop(0, n, body, 0)
    obuf[...] = o32[...].astype(obuf.dtype)
    oc = pltpu.make_async_copy(obuf, o_hbm, osem.at[0])
    oc.start()
    oc.wait()


@jax.jit
def pallas_standalone__gqa_softmax__decode_kernel(
    q: jax.Array,
    k: jax.Array,
    v: jax.Array,
):
    B, Hq, Sq, D = q.shape
    _, Hkv, Sk, _ = k.shape
    rep = Hq // Hkv
    M = rep * Sq
    N = B * Hkv
    scale = D ** -0.5
    ahead = 2
    nbuf = ahead + 2
    assert N > nbuf and Sk % 16 == 0 and Sk >= 4 * _TA
    if Sk == 4096:
        ksizes = tuple(8 * u for u in _K_UNITS_4096)
        vsizes = tuple(8 * u for u in _V_UNITS_4096)
        lead = _V_LEAD_4096
    else:
        ksizes = vsizes = _uniform(Sk, 192)
        lead = 0
    q2 = q.reshape(N * M, D)
    k2 = k.reshape(N * Sk, D)
    v2 = v.reshape(N * Sk, D)
    out = pl.pallas_call(
        functools.partial(_kernel, n=N, m=M, sk=Sk, nbuf=nbuf, ahead=ahead,
                          ksizes=ksizes, vsizes=vsizes, lead=lead,
                          off=8 * _OFF, scale=scale),
        in_specs=[pl.BlockSpec(memory_space=pl.ANY)] * 3,
        out_specs=pl.BlockSpec(memory_space=pl.ANY),
        out_shape=jax.ShapeDtypeStruct((N * M, D), q.dtype),
        scratch_shapes=[
            pltpu.VMEM((N * M, D), q.dtype),
            pltpu.VMEM((N * M, D), jnp.float32),
            pltpu.VMEM((nbuf, Sk, D), k.dtype),
            pltpu.VMEM((nbuf, Sk, D), v.dtype),
            pltpu.VMEM((N * M, D), jnp.float32),
            pltpu.VMEM((N * M, D), q.dtype),
            pltpu.SemaphoreType.DMA((1,)),
            pltpu.SemaphoreType.DMA((nbuf,)),
            pltpu.SemaphoreType.DMA((nbuf,)),
            pltpu.SemaphoreType.DMA((1,)),
        ],
        compiler_params=pltpu.CompilerParams(
            vmem_limit_bytes=64 * 1024 * 1024),
    )(q2, k2, v2)
    return out.reshape(B, Hq, Sq, D)
```

```python
import functools

import jax
import jax.numpy as jnp
from jax import lax
import jax.experimental.pallas as pl
import jax.experimental.pallas.tpu as pltpu

_K_UNITS_4096 = (
    30, 1, 1, 30, 1, 1, 24, 7, 1, 24, 7, 1, 25, 6, 1, 30, 1, 1, 30, 1, 1, 27, 4, 1,
    30, 1, 1, 30, 1, 1, 30, 1, 1, 30, 1, 1, 30, 1, 1, 30, 1, 1, 30, 1, 1, 30, 1, 1)
_V_UNITS_4096 = (
    5, 24, 3, 3, 26, 2, 5, 25, 3, 5, 24, 2, 4, 26, 3, 4, 24, 3, 5, 26, 1, 3, 27, 2,
    5, 24, 1, 8, 23, 4, 1, 28, 5, 6, 21, 3, 5, 24, 3, 9, 20, 3, 3, 25, 5, 1, 27, 3)
_V_LEAD_4096 = 10
_OFF = 13
_TA = 128


def _pieces(sizes):
    out = []
    o = 0
    for r in sizes:
        out.append((o, r))
        o += r
    return out


def _uniform(total, size):
    out = []
    while sum(out) < total:
        out.append(min(size, total - sum(out)))
    return tuple(out)


def _kernel(q_hbm, k_hbm, v_hbm, o_hbm, qbuf, q32, kbuf, vbuf, o32, obuf,
            qsem, ksem, vsem, osem, *, n, m, sk, nbuf, ahead, ksizes, vsizes,
            lead, off, scale):
    kp, vp = _pieces(ksizes), _pieces(vsizes)
    npc = len(kp)
    body_rows = sk - off
    ta = _TA
    d = kbuf.shape[-1]

    def slot_of(g):
        return g % nbuf if isinstance(g, int) else lax.rem(g, nbuf)

    def start(hbm, buf, sem, queue, g, piece, trunc):
        o, r = piece
        if trunc:
            r = min(r, body_rows - o)
            if r <= 0:
                return
        slot = slot_of(g)
        src = g * sk + off + o
        if not isinstance(src, int):
            src = pl.multiple_of(src, 8)
        pltpu.make_async_copy(hbm.at[pl.ds(src, r)],
                              buf.at[slot, pl.ds(o, r)],
                              sem.at[slot]).start(priority=queue)

    def issue(g, last):
        for i in range(npc):
            start(k_hbm, kbuf, ksem, 0, g, kp[i], last)
            if i + lead < npc:
                start(v_hbm, vbuf, vsem, 1, g, vp[i + lead], last)
            elif not last:
                start(v_hbm, vbuf, vsem, 1, g + 1, vp[i + lead - npc], False)

    qc = pltpu.make_async_copy(q_hbm, qbuf, qsem.at[0])
    qc.start()
    ls = nbuf - 1
    k0c = pltpu.make_async_copy(k_hbm.at[pl.ds(0, off)],
                                kbuf.at[ls, pl.ds(body_rows, off)], ksem.at[ls])
    v0c = pltpu.make_async_copy(v_hbm.at[pl.ds(0, off)],
                                vbuf.at[ls, pl.ds(body_rows, off)], vsem.at[ls])
    k0c.start(priority=0)
    v0c.start(priority=1)
    for i in range(lead):
        start(v_hbm, vbuf, vsem, 1, 0, vp[i], False)
    for j in range(ahead):
        issue(j, False)
    qc.wait()
    q32[...] = qbuf[...].astype(jnp.float32)
    k0c.wait()
    v0c.wait()
    kbuf[ls, pl.ds(sk - ta, ta - off), :] = jnp.zeros((ta - off, d), kbuf.dtype)
    vbuf[ls, pl.ds(sk - ta, ta - off), :] = jnp.zeros((ta - off, d), vbuf.dtype)

    lane = lax.broadcasted_iota(jnp.int32, (m, ta), 1)
    row = lax.broadcasted_iota(jnp.int32, (ta, d), 0)
    neg = jnp.float32(-jnp.inf)

    def wait_group(buf, sem, slot, h):
        a = buf.at[slot, pl.ds(0, body_rows)]
        pltpu.make_async_copy(a, a, sem.at[slot]).wait()

        @pl.when(h < n - 1)
        def _():
            b = buf.at[slot, pl.ds(body_rows, off)]
            pltpu.make_async_copy(b, b, sem.at[slot]).wait()

    def body(h, carry):
        slot = lax.rem(h, nbuf)
        pslot = lax.rem(h + nbuf - 1, nbuf)
        nxt = h + ahead

        @pl.when(nxt < n - 1)
        def _():
            issue(nxt, False)

        @pl.when(nxt == n - 1)
        def _():
            issue(nxt, True)

        q = q32[pl.ds(h * m, m), :].astype(kbuf.dtype)
        wait_group(kbuf, ksem, slot, h)
        dn = (((1,), (1,)), ((), ()))
        sa = lax.dot_general(q, kbuf[pslot, pl.ds(sk - ta, ta), :], dn,
                             preferred_element_type=jnp.float32)
        sb = lax.dot_general(q, kbuf[slot, pl.ds(0, sk - ta), :], dn,
                             preferred_element_type=jnp.float32)
        sc = lax.dot_general(q, kbuf[slot, pl.ds(sk - ta, ta), :], dn,
                             preferred_element_type=jnp.float32)
        sa = jnp.where(lane >= ta - off, sa * scale, neg)
        sb = sb * scale
        sc = jnp.where(lane < ta - off, sc * scale, neg)
        mx = jnp.maximum(jnp.max(sb, axis=-1, keepdims=True),
                         jnp.max(jnp.maximum(sa, sc), axis=-1, keepdims=True))
        pa = jnp.exp(sa - mx)
        pb = jnp.exp(sb - mx)
        pc = jnp.exp(sc - mx)
        l = (jnp.sum(pb, axis=-1, keepdims=True)
             + jnp.sum(pa + pc, axis=-1, keepdims=True))
        wait_group(vbuf, vsem, slot, h)
        dt = vbuf.dtype
        acc = jnp.dot(pb.astype(dt), vbuf[slot, pl.ds(0, sk - ta), :],
                      preferred_element_type=jnp.float32)
        va = vbuf[pslot, pl.ds(sk - ta, ta), :].astype(jnp.float32)
        vc = vbuf[slot, pl.ds(sk - ta, ta), :].astype(jnp.float32)
        va = jnp.where(row >= ta - off, va, 0.0).astype(dt)
        vc = jnp.where(row < ta - off, vc, 0.0).astype(dt)
        acc = acc + jnp.dot(pa.astype(dt), va, preferred_element_type=jnp.float32)
        acc = acc + jnp.dot(pc.astype(dt), vc, preferred_element_type=jnp.float32)
        o32[pl.ds(h * m, m), :] = acc / l
        return carry

    lax.fori_loop(0, n, body, 0)
    obuf[...] = o32[...].astype(obuf.dtype)
    oc = pltpu.make_async_copy(obuf, o_hbm, osem.at[0])
    oc.start()
    oc.wait()


@jax.jit
def pallas_standalone__gqa_softmax__decode_kernel(
    q: jax.Array,
    k: jax.Array,
    v: jax.Array,
):
    B, Hq, Sq, D = q.shape
    _, Hkv, Sk, _ = k.shape
    rep = Hq // Hkv
    M = rep * Sq
    N = B * Hkv
    scale = D ** -0.5
    ahead = 2
    nbuf = ahead + 2
    assert N > nbuf and Sk % 16 == 0 and Sk >= 4 * _TA
    if Sk == 4096:
        ksizes = tuple(8 * u for u in _K_UNITS_4096)
        vsizes = tuple(8 * u for u in _V_UNITS_4096)
        lead = _V_LEAD_4096
    else:
        ksizes = vsizes = _uniform(Sk, 192)
        lead = 0
    q2 = q.reshape(N * M, D)
    k2 = k.reshape(N * Sk, D)
    v2 = v.reshape(N * Sk, D)
    out = pl.pallas_call(
        functools.partial(_kernel, n=N, m=M, sk=Sk, nbuf=nbuf, ahead=ahead,
                          ksizes=ksizes, vsizes=vsizes, lead=lead,
                          off=8 * _OFF, scale=scale),
        in_specs=[pl.BlockSpec(memory_space=pl.ANY)] * 3,
        out_specs=pl.BlockSpec(memory_space=pl.ANY),
        out_shape=jax.ShapeDtypeStruct((N * M, D), q.dtype),
        scratch_shapes=[
            pltpu.VMEM((N * M, D), q.dtype),
            pltpu.VMEM((N * M, D), jnp.float32),
            pltpu.VMEM((nbuf, Sk, D), k.dtype),
            pltpu.VMEM((nbuf, Sk, D), v.dtype),
            pltpu.VMEM((N * M, D), jnp.float32),
            pltpu.VMEM((N * M, D), q.dtype),
            pltpu.SemaphoreType.DMA((1,)),
            pltpu.SemaphoreType.DMA((nbuf,)),
            pltpu.SemaphoreType.DMA((nbuf,)),
            pltpu.SemaphoreType.DMA((1,)),
        ],
        compiler_params=pltpu.CompilerParams(
            vmem_limit_bytes=64 * 1024 * 1024),
    )(q2, k2, v2)
    return out.reshape(B, Hq, Sq, D)
```

```python
import functools

import jax
import jax.numpy as jnp
from jax import lax
import jax.experimental.pallas as pl
import jax.experimental.pallas.tpu as pltpu


def _kernel(q_hbm, k_hbm, v_hbm, o_hbm, qbuf, q32, qcur, kbuf, vbuf, o32, obuf,
            qsem, ksem, vsem, osem, *, n, m, sk, C, S, rc, r, nbuf, ahead, lead,
            scale):
    nj = sk // rc
    nc = S * nj
    nset = n // C
    nstep = nset * nj
    npc = rc // r
    d = kbuf.shape[-1]
    cm = C * m
    dt = kbuf.dtype

    def start(hbm, buf, sem, queue, t, i):
        o = i * r
        if isinstance(t, int):
            g, c = divmod(t, nc)
            slot = t % nbuf
            src = c * rc + o
        else:
            g = lax.div(t, nc)
            slot = lax.rem(t, nbuf)
            src = pl.multiple_of(lax.rem(t, nc) * rc + o, r)
        pltpu.make_async_copy(hbm.at[pl.ds(g * C, C), pl.ds(src, r), :],
                              buf.at[slot, :, pl.ds(o, r), :],
                              sem.at[slot]).start(priority=queue)

    def issue(t, last):
        for i in range(npc):
            start(k_hbm, kbuf, ksem, 0, t, i)
            if i + lead < npc:
                start(v_hbm, vbuf, vsem, 1, t, i + lead)
            elif not last:
                start(v_hbm, vbuf, vsem, 1, t + 1, i + lead - npc)

    qc = pltpu.make_async_copy(q_hbm, qbuf, qsem.at[0])
    qc.start()
    for i in range(lead):
        start(v_hbm, vbuf, vsem, 1, 0, i)
    for t in range(ahead):
        issue(t, False)
    qc.wait()
    q32[...] = qbuf[...].astype(jnp.float32)

    rows_s = lax.broadcasted_iota(jnp.int32, (cm, rc), 0)
    rows_o = lax.broadcasted_iota(jnp.int32, (cm, d), 0)
    dn = (((1,), (1,)), ((), ()))

    def set_body(u, carry):
        h0 = lax.div(u, S) * (C * S) + lax.rem(u, S)
        for c in range(C):
            qcur[pl.ds(c * m, m), :] = q32[pl.ds((h0 + c * S) * m, m), :]
        q = qcur[...].astype(dt)

        def step(j, st):
            mx, l, acc = st
            t = u * nj + j
            slot = lax.rem(t, nbuf)
            nxt = t + ahead

            @pl.when(nxt < nstep - 1)
            def _():
                issue(nxt, False)

            @pl.when(nxt == nstep - 1)
            def _():
                issue(nxt, True)

            pltpu.make_async_copy(kbuf.at[slot], kbuf.at[slot], ksem.at[slot]).wait()
            s = None
            for c in range(C):
                sc = lax.dot_general(q, kbuf[slot, c], dn,
                                     preferred_element_type=jnp.float32)
                s = sc if s is None else jnp.where(rows_s >= c * m, sc, s)
            s = s * scale
            mn = jnp.maximum(mx, jnp.max(s, axis=-1, keepdims=True))
            ms = jnp.where(mn == -jnp.inf, 0.0, mn)
            alpha = jnp.exp(mx - ms)
            p = jnp.exp(s - ms)
            l = alpha * l + jnp.sum(p, axis=-1, keepdims=True)
            pb = p.astype(dt)
            pltpu.make_async_copy(vbuf.at[slot], vbuf.at[slot], vsem.at[slot]).wait()
            o = None
            for c in range(C):
                oc = jnp.dot(pb, vbuf[slot, c], preferred_element_type=jnp.float32)
                o = oc if o is None else jnp.where(rows_o >= c * m, oc, o)
            return mn, l, alpha * acc + o

        init = (jnp.full((cm, 1), -jnp.inf, jnp.float32),
                jnp.zeros((cm, 1), jnp.float32),
                jnp.zeros((cm, d), jnp.float32))
        _, l, acc = lax.fori_loop(0, nj, step, init)
        res = acc / l
        for c in range(C):
            o32[pl.ds((h0 + c * S) * m, m), :] = res[c * m:(c + 1) * m, :]
        return carry

    lax.fori_loop(0, nset, set_body, 0)
    obuf[...] = o32[...].astype(obuf.dtype)
    oc = pltpu.make_async_copy(obuf, o_hbm, osem.at[0])
    oc.start()
    oc.wait()


@jax.jit
def pallas_standalone__gqa_softmax__decode_kernel(
    q: jax.Array,
    k: jax.Array,
    v: jax.Array,
):
    B, Hq, Sq, D = q.shape
    _, Hkv, Sk, _ = k.shape
    rep = Hq // Hkv
    M = rep * Sq
    N = B * Hkv
    scale = D ** -0.5
    S = 2 if N % 16 == 0 else 1
    C = next(c for c in (8, 4, 2, 1) if N % (c * S) == 0)
    r = 16
    rc = next(x for x in (512, 256, 128, 64, 32, 16) if Sk % x == 0)
    lead = (3 * (rc // r)) // 4
    ahead = 2
    nbuf = ahead + 2
    assert (N // C) * (Sk // rc) > ahead
    q2 = q.reshape(N * M, D)
    k2 = k.reshape(N // S, S * Sk, D)
    v2 = v.reshape(N // S, S * Sk, D)
    out = pl.pallas_call(
        functools.partial(_kernel, n=N, m=M, sk=Sk, C=C, S=S, rc=rc, r=r,
                          nbuf=nbuf, ahead=ahead, lead=lead, scale=scale),
        in_specs=[pl.BlockSpec(memory_space=pl.ANY)] * 3,
        out_specs=pl.BlockSpec(memory_space=pl.ANY),
        out_shape=jax.ShapeDtypeStruct((N * M, D), q.dtype),
        scratch_shapes=[
            pltpu.VMEM((N * M, D), q.dtype),
            pltpu.VMEM((N * M, D), jnp.float32),
            pltpu.VMEM((C * M, D), jnp.float32),
            pltpu.VMEM((nbuf, C, rc, D), k.dtype),
            pltpu.VMEM((nbuf, C, rc, D), v.dtype),
            pltpu.VMEM((N * M, D), jnp.float32),
            pltpu.VMEM((N * M, D), q.dtype),
            pltpu.SemaphoreType.DMA((1,)),
            pltpu.SemaphoreType.DMA((nbuf,)),
            pltpu.SemaphoreType.DMA((nbuf,)),
            pltpu.SemaphoreType.DMA((1,)),
        ],
        compiler_params=pltpu.CompilerParams(
            vmem_limit_bytes=64 * 1024 * 1024),
    )(q2, k2, v2)
    return out.reshape(B, Hq, Sq, D)
```

```python
import functools

import jax
import jax.numpy as jnp
from jax import lax
import jax.experimental.pallas as pl
import jax.experimental.pallas.tpu as pltpu


def _kernel(q_hbm, k_hbm, v_hbm, o_hbm, qbuf, q32, qcur, kbuf, vbuf, o32, obuf,
            qsem, ksem, vsem, osem, *, n, m, sk, C, S, rc, r, nbuf, ahead, lead,
            scale):
    nj = sk // rc
    nc = S * nj
    nset = n // C
    nstep = nset * nj
    npc = rc // r
    d = kbuf.shape[-1]
    cm = C * m
    dt = kbuf.dtype

    def start(hbm, buf, sem, queue, t, i):
        o = i * r
        if isinstance(t, int):
            g, c = divmod(t, nc)
            slot = t % nbuf
            src = c * rc + o
        else:
            g = lax.div(t, nc)
            slot = lax.rem(t, nbuf)
            src = pl.multiple_of(lax.rem(t, nc) * rc + o, r)
        pltpu.make_async_copy(hbm.at[pl.ds(g * C, C), pl.ds(src, r), :],
                              buf.at[slot, :, pl.ds(o, r), :],
                              sem.at[slot]).start(priority=queue)

    def issue(t, last):
        for i in range(npc):
            start(k_hbm, kbuf, ksem, 0, t, i)
            if i + lead < npc:
                start(v_hbm, vbuf, vsem, 1, t, i + lead)
            elif not last:
                start(v_hbm, vbuf, vsem, 1, t + 1, i + lead - npc)

    qc = pltpu.make_async_copy(q_hbm, qbuf, qsem.at[0])
    qc.start()
    for i in range(lead):
        start(v_hbm, vbuf, vsem, 1, 0, i)
    for t in range(ahead):
        issue(t, False)
    qc.wait()
    q32[...] = qbuf[...].astype(jnp.float32)

    rows_s = lax.broadcasted_iota(jnp.int32, (cm, rc), 0)
    rows_o = lax.broadcasted_iota(jnp.int32, (cm, d), 0)
    dn = (((1,), (1,)), ((), ()))

    def set_body(u, carry):
        h0 = lax.div(u, S) * (C * S) + lax.rem(u, S)
        for c in range(C):
            qcur[pl.ds(c * m, m), :] = q32[pl.ds((h0 + c * S) * m, m), :]
        q = qcur[...].astype(dt)

        def step(j, st):
            mx, l, acc = st
            t = u * nj + j
            slot = lax.rem(t, nbuf)
            nxt = t + ahead

            @pl.when(nxt < nstep - 1)
            def _():
                issue(nxt, False)

            @pl.when(nxt == nstep - 1)
            def _():
                issue(nxt, True)

            pltpu.make_async_copy(kbuf.at[slot], kbuf.at[slot], ksem.at[slot]).wait()
            s = None
            for c in range(C):
                sc = lax.dot_general(q, kbuf[slot, c], dn,
                                     preferred_element_type=jnp.float32)
                s = sc if s is None else jnp.where(rows_s >= c * m, sc, s)
            s = s * scale
            mn = jnp.maximum(mx, jnp.max(s, axis=-1, keepdims=True))
            ms = jnp.where(mn == -jnp.inf, 0.0, mn)
            alpha = jnp.exp(mx - ms)
            p = jnp.exp(s - ms)
            l = alpha * l + jnp.sum(p, axis=-1, keepdims=True)
            pb = p.astype(dt)
            pltpu.make_async_copy(vbuf.at[slot], vbuf.at[slot], vsem.at[slot]).wait()
            o = None
            for c in range(C):
                oc = jnp.dot(pb, vbuf[slot, c], preferred_element_type=jnp.float32)
                o = oc if o is None else jnp.where(rows_o >= c * m, oc, o)
            return mn, l, alpha * acc + o

        init = (jnp.full((cm, 1), -jnp.inf, jnp.float32),
                jnp.zeros((cm, 1), jnp.float32),
                jnp.zeros((cm, d), jnp.float32))
        _, l, acc = lax.fori_loop(0, nj, step, init)
        res = acc / l
        for c in range(C):
            o32[pl.ds((h0 + c * S) * m, m), :] = res[c * m:(c + 1) * m, :]
        return carry

    lax.fori_loop(0, nset, set_body, 0)
    obuf[...] = o32[...].astype(obuf.dtype)
    oc = pltpu.make_async_copy(obuf, o_hbm, osem.at[0])
    oc.start()
    oc.wait()


@jax.jit
def pallas_standalone__gqa_softmax__decode_kernel(
    q: jax.Array,
    k: jax.Array,
    v: jax.Array,
):
    B, Hq, Sq, D = q.shape
    _, Hkv, Sk, _ = k.shape
    rep = Hq // Hkv
    M = rep * Sq
    N = B * Hkv
    scale = D ** -0.5
    ahead = 2
    nbuf = ahead + 2
    C = next(c for c in (8, 4, 2, 1) if N % c == 0)
    S = N // C
    r = 16
    rc = next(x for x in (512, 256, 128, 64, 32, 16)
              if Sk % x == 0 and S * (Sk // x) > ahead)
    lead = min(26, rc // r - 1)
    q2 = q.reshape(N * M, D)
    k2 = k.reshape(N // S, S * Sk, D)
    v2 = v.reshape(N // S, S * Sk, D)
    out = pl.pallas_call(
        functools.partial(_kernel, n=N, m=M, sk=Sk, C=C, S=S, rc=rc, r=r,
                          nbuf=nbuf, ahead=ahead, lead=lead, scale=scale),
        in_specs=[pl.BlockSpec(memory_space=pl.ANY)] * 3,
        out_specs=pl.BlockSpec(memory_space=pl.ANY),
        out_shape=jax.ShapeDtypeStruct((N * M, D), q.dtype),
        scratch_shapes=[
            pltpu.VMEM((N * M, D), q.dtype),
            pltpu.VMEM((N * M, D), jnp.float32),
            pltpu.VMEM((C * M, D), jnp.float32),
            pltpu.VMEM((nbuf, C, rc, D), k.dtype),
            pltpu.VMEM((nbuf, C, rc, D), v.dtype),
            pltpu.VMEM((N * M, D), jnp.float32),
            pltpu.VMEM((N * M, D), q.dtype),
            pltpu.SemaphoreType.DMA((1,)),
            pltpu.SemaphoreType.DMA((nbuf,)),
            pltpu.SemaphoreType.DMA((nbuf,)),
            pltpu.SemaphoreType.DMA((1,)),
        ],
        compiler_params=pltpu.CompilerParams(
            vmem_limit_bytes=64 * 1024 * 1024),
    )(q2, k2, v2)
    return out.reshape(B, Hq, Sq, D)
```

```python
import functools

import jax
import jax.numpy as jnp
from jax import lax
import jax.experimental.pallas as pl
import jax.experimental.pallas.tpu as pltpu


def _kernel(q_hbm, k_hbm, v_hbm, o_hbm, qbuf, q32, qcur, kbuf, vbuf, o32, obuf,
            qsem, ksem, vsem, osem, *, n, m, sk, C, rc, r, vsub, nbuf, ahead,
            lead, scale):
    nj = sk // rc
    nset = n // C
    nstep = nset * nj
    npc = rc // r
    nsv = len(vsub)
    d = kbuf.shape[-1]
    cm = C * m
    dt = kbuf.dtype

    def start(hbm, buf, queue, t, i):
        o = i * r
        if isinstance(t, int):
            slot = t % nbuf
            src = t * rc + o
        else:
            slot = lax.rem(t, nbuf)
            src = pl.multiple_of(t * rc + o, r)
        if queue == 0:
            sem = ksem.at[slot]
        else:
            b = [x for x, (lo, hi) in enumerate(vsub) if lo <= o < hi][0]
            sem = vsem.at[slot * nsv + b]
        pltpu.make_async_copy(hbm.at[:, pl.ds(src, r), :],
                              buf.at[slot, :, pl.ds(o, r), :],
                              sem).start(priority=queue)

    def issue(t, last):
        for i in range(npc):
            start(k_hbm, kbuf, 0, t, i)
            if i + lead < npc:
                start(v_hbm, vbuf, 1, t, i + lead)
            elif not last:
                start(v_hbm, vbuf, 1, t + 1, i + lead - npc)

    qc = pltpu.make_async_copy(q_hbm, qbuf, qsem.at[0])
    qc.start()
    for i in range(lead):
        start(v_hbm, vbuf, 1, 0, i)
    for t in range(ahead):
        issue(t, False)
    qc.wait()
    q32[...] = qbuf[...].astype(jnp.float32)

    rows_s = lax.broadcasted_iota(jnp.int32, (cm, rc), 0)
    rows_o = lax.broadcasted_iota(jnp.int32, (cm, d), 0)
    dn = (((1,), (1,)), ((), ()))

    def set_body(u, carry):
        for c in range(C):
            qcur[pl.ds(c * m, m), :] = q32[pl.ds((c * nset + u) * m, m), :]
        q = qcur[...].astype(dt)

        def step(j, st):
            mx, l, acc = st
            t = u * nj + j
            slot = lax.rem(t, nbuf)
            nxt = t + ahead

            @pl.when(nxt < nstep - 1)
            def _():
                issue(nxt, False)

            @pl.when(nxt == nstep - 1)
            def _():
                issue(nxt, True)

            pltpu.make_async_copy(kbuf.at[slot], kbuf.at[slot], ksem.at[slot]).wait()
            s = None
            for c in range(C):
                sc = lax.dot_general(q, kbuf[slot, c], dn,
                                     preferred_element_type=jnp.float32)
                s = sc if s is None else jnp.where(rows_s >= c * m, sc, s)
            s = s * scale
            mn = jnp.maximum(mx, jnp.max(s, axis=-1, keepdims=True))
            ms = jnp.where(mn == -jnp.inf, 0.0, mn)
            alpha = jnp.exp(mx - ms)
            p = jnp.exp(s - ms)
            l = alpha * l + jnp.sum(p, axis=-1, keepdims=True)
            pb = p.astype(dt)
            acc = alpha * acc
            for b, (lo, hi) in enumerate(vsub):
                vv = vbuf.at[slot, :, pl.ds(lo, hi - lo), :]
                pltpu.make_async_copy(vv, vv, vsem.at[slot * nsv + b]).wait()
                o = None
                for c in range(C):
                    oc = jnp.dot(pb[:, lo:hi], vbuf[slot, c, pl.ds(lo, hi - lo), :],
                                 preferred_element_type=jnp.float32)
                    o = oc if o is None else jnp.where(rows_o >= c * m, oc, o)
                acc = acc + o
            return mn, l, acc

        init = (jnp.full((cm, 1), -jnp.inf, jnp.float32),
                jnp.zeros((cm, 1), jnp.float32),
                jnp.zeros((cm, d), jnp.float32))
        _, l, acc = lax.fori_loop(0, nj, step, init)
        res = acc / l
        for c in range(C):
            o32[pl.ds((c * nset + u) * m, m), :] = res[c * m:(c + 1) * m, :]
        return carry

    lax.fori_loop(0, nset, set_body, 0)
    obuf[...] = o32[...].astype(obuf.dtype)
    oc = pltpu.make_async_copy(obuf, o_hbm, osem.at[0])
    oc.start()
    oc.wait()


@jax.jit
def pallas_standalone__gqa_softmax__decode_kernel(
    q: jax.Array,
    k: jax.Array,
    v: jax.Array,
):
    B, Hq, Sq, D = q.shape
    _, Hkv, Sk, _ = k.shape
    rep = Hq // Hkv
    M = rep * Sq
    N = B * Hkv
    scale = D ** -0.5
    ahead = 2
    nbuf = ahead + 2
    C = next(c for c in (8, 4, 2, 1) if N % c == 0)
    r = 16
    rc = next(x for x in (512, 256, 128, 64, 32, 16)
              if Sk % x == 0 and (N // C) * (Sk // x) > ahead)
    lead = min(26, rc // r - 1)
    vsub = ((0, rc - 128), (rc - 128, rc)) if rc >= 256 else ((0, rc),)
    q2 = q.reshape(N * M, D)
    k2 = k.reshape(C, (N // C) * Sk, D)
    v2 = v.reshape(C, (N // C) * Sk, D)
    out = pl.pallas_call(
        functools.partial(_kernel, n=N, m=M, sk=Sk, C=C, rc=rc, r=r, vsub=vsub,
                          nbuf=nbuf, ahead=ahead, lead=lead, scale=scale),
        in_specs=[pl.BlockSpec(memory_space=pl.ANY)] * 3,
        out_specs=pl.BlockSpec(memory_space=pl.ANY),
        out_shape=jax.ShapeDtypeStruct((N * M, D), q.dtype),
        scratch_shapes=[
            pltpu.VMEM((N * M, D), q.dtype),
            pltpu.VMEM((N * M, D), jnp.float32),
            pltpu.VMEM((C * M, D), jnp.float32),
            pltpu.VMEM((nbuf, C, rc, D), k.dtype),
            pltpu.VMEM((nbuf, C, rc, D), v.dtype),
            pltpu.VMEM((N * M, D), jnp.float32),
            pltpu.VMEM((N * M, D), q.dtype),
            pltpu.SemaphoreType.DMA((1,)),
            pltpu.SemaphoreType.DMA((nbuf,)),
            pltpu.SemaphoreType.DMA((nbuf * len(vsub),)),
            pltpu.SemaphoreType.DMA((1,)),
        ],
        compiler_params=pltpu.CompilerParams(
            vmem_limit_bytes=64 * 1024 * 1024),
    )(q2, k2, v2)
    return out.reshape(B, Hq, Sq, D)
```
